```python
import os as _os
_os.environ.setdefault("JAX_PLATFORMS", "cpu")
import jax
import jax.numpy as jnp

def _softmax(x, axis=-1):
    return jax.nn.softmax(x, axis=axis)
def _gelu(x):
    return jax.nn.gelu(x, approximate=True)
def _silu(x):
    return jax.nn.silu(x)
def _sigmoid(x):
    return jax.nn.sigmoid(x)
def _layernorm(x, axis=-1, eps=1e-5):
    m = jnp.mean(x, axis=axis, keepdims=True)
    v = jnp.var(x, axis=axis, keepdims=True)
    return (x - m) / jnp.sqrt(v + eps)
def _scatter_add(tgt, idx, src, axis=0):
    return tgt.at[idx].add(src)
def _segment_sum(src, seg, n):
    return jax.ops.segment_sum(src, seg, n)
class _Rng:
    def __init__(self, key):
        self._k = key
    def _next(self):
        self._k, sub = jax.random.split(self._k)
        return sub
    def normal(self, shape):
        return jax.random.normal(self._next(), shape, dtype=jnp.bfloat16)
    def randint(self, lo, hi, shape):
        return jax.random.randint(self._next(), shape, lo, hi, dtype=jnp.int32)
    def uniform(self, shape, lo=0.0, hi=1.0):
        return jax.random.uniform(self._next(), shape, jnp.bfloat16, lo, hi)
    def permutation(self, n):
        return jax.random.permutation(self._next(), n)


kernel_name = 'recurrent_scan__grouped_kv_mqa__mixer_s_mlp__prompt'

def setup_inputs():
    _rng = _Rng(jax.random.key(int.from_bytes(__import__("os").urandom(4), "little")))
    _w = (lambda a: (lambda t: t.astype(jnp.bfloat16) if jnp.issubdtype(t.dtype, jnp.floating) else t)(jnp.asarray(a)))
    def _A_setup():
        B, S, D, H = 1, 2048, 512, 32
        Dh = D // H
        return {
            "x": _w((lambda *s: _rng.normal(s) * 0.05)(B, S, D)),
            "wq": _w((lambda *s: _rng.normal(s) * 0.05)(D, H * Dh)),
            "wk": _w((lambda *s: _rng.normal(s) * 0.05)(D, Dh)),
            "wv": _w((lambda *s: _rng.normal(s) * 0.05)(D, Dh)),
            "wo": _w((lambda *s: _rng.normal(s) * 0.05)(H * Dh, D)),
        }
    _A_in = _A_setup()

    def _B_setup():
        B, S, D, F = 1, 2048, 512, 1792
        return {
            "x":  _w((lambda *s: _rng.normal(s) * 0.05)(B, S, D)),
            "w1": _w((lambda *s: _rng.normal(s) * 0.8)(D, D) * (D ** -0.5)),
            "w2": _w((lambda *s: _rng.normal(s) * 0.8)(D, D) * (D ** -0.5)),
            "w3": _w((lambda *s: _rng.normal(s) * 0.8)(D, F) * (D ** -0.5)),
            "w4": _w((lambda *s: _rng.normal(s) * 0.8)(F, D) * (F ** -0.5)),
        }
    _B_in = _B_setup()

    return {
        "A_x": _A_in["x"],
        "A_wq": _A_in["wq"],
        "A_wk": _A_in["wk"],
        "A_wv": _A_in["wv"],
        "A_wo": _A_in["wo"],
        "B_x": _B_in["x"],
        "B_w1": _B_in["w1"],
        "B_w2": _B_in["w2"],
        "B_w3": _B_in["w3"],
        "B_w4": _B_in["w4"],
    }

def reference(A_x, A_wq, A_wk, A_wv, A_wo, B_x, B_w1, B_w2, B_w3, B_w4):
    def _A_ref(x, wq, wk, wv, wo):
        B, S, D = x.shape
        H = 32
        Dh = D // H
        q = (lambda x, *d: x.transpose(*d))((x @ wq).reshape(B, S, H, Dh), 0, 2, 1, 3)
        k = x @ wk
        v = x @ wv
        scores = jnp.einsum("bhqd,bkd->bhqk", q, k) * (Dh ** -0.5)
        p = _softmax(scores, axis=-1)
        o = jnp.einsum("bhqk,bkd->bhqd", p, v)
        return (lambda x, *d: x.transpose(*d))(o, 0, 2, 1, 3).reshape(B, S, H * Dh) @ wo

    def _B_ref(x, w1, w2, w3, w4):
        B, S, D = x.shape
        h = _gelu(_layernorm(x, axis=-1) @ w1)
        c = D // 4
        g0 = jnp.pad(h[:, :, 0*c:1*c], ((0, 0), (1, 0), (0, 0)))[:, :S, :]
        g1 = jnp.pad(h[:, :, 1*c:2*c], ((0, 0), (0, 1), (0, 0)))[:, 1:, :]
        g2 = jnp.pad(h[:, :, 2*c:3*c], ((0, 0), (2, 0), (0, 0)))[:, :S, :]
        g3 = jnp.pad(h[:, :, 3*c:   ], ((0, 0), (0, 2), (0, 0)))[:, 2:, :]
        hs = jnp.concatenate([g0, g1, g2, g3], axis=-1) @ w2
        x1 = x + hs
        h2 = _gelu(_layernorm(x1, axis=-1) @ w3) @ w4
        return x1 + h2

    x = A_x
    xn = _layernorm(x, axis=-1)
    s = _A_ref(xn, A_wq, A_wk, A_wv, A_wo)
    g = _silu(_B_ref(xn, B_w1, B_w2, B_w3, B_w4))
    return x + s * g
```

```python
import math

import jax
import jax.numpy as jnp
import jax.experimental.pallas as pl
import jax.experimental.pallas.tpu as pltpu

S, D, H, DH, F = 2048, 512, 32, 16, 1792
TQ = 512
CK = 128
TR = 256
FC = 256
UNROLL = 4
LAG = 3
QSCALE = (DH ** -0.5) * math.log2(math.e)
F32, BF16 = jnp.float32, jnp.bfloat16


def _dot(a, b):
    return jnp.dot(a, b, preferred_element_type=F32)


def _dot_nt(a, b):
    return jax.lax.dot_general(a, b, (((1,), (1,)), ((), ())), preferred_element_type=F32)


def _ln(x):
    m = jnp.mean(x, axis=-1, keepdims=True)
    d = x - m
    v = jnp.mean(d * d, axis=-1, keepdims=True)
    return d * jax.lax.rsqrt(v + 1e-5)


def _gelu(x):
    c = math.sqrt(2.0 / math.pi)
    u = x * (c + (c * 0.044715) * (x * x))
    return (0.5 * x) * (1.0 + jnp.tanh(u))


def _fold8(x, op):
    r = x[0:8]
    for i in range(1, x.shape[0] // 8):
        r = op(r, x[8 * i:8 * i + 8])
    return r


def _kernel(x_ref, wq_ref, wk_ref, wv_ref, wo_ref, w1_ref, w2_ref, w3_ref, w4_ref, o_ref,
            wt_ref, xn_ref, h_ref, g_ref, qt_ref, k_ref, vt_ref, s_ref, ot_ref):
    wt_ref[0:D, :] = wq_ref[...].astype(F32).T.astype(BF16)
    wt_ref[D:D + DH, :] = wk_ref[...].astype(F32).T.astype(BF16)
    wt_ref[D + DH:D + 2 * DH, :] = wv_ref[...].astype(F32).T.astype(BF16)
    h_ref[0:8, :] = jnp.zeros((8, D), F32)
    h_ref[S + 8:S + 16, :] = jnp.zeros((8, D), F32)

    def p1(t, c):
        r0 = pl.multiple_of(t * TR, TR)
        xn = _ln(x_ref[pl.ds(r0, TR), :].astype(F32))
        xn_ref[pl.ds(r0, TR), :] = xn
        qkv = _dot_nt(wt_ref[...], xn.astype(BF16))
        qt_ref[:, pl.ds(r0, TR)] = (qkv[0:D] * QSCALE).astype(BF16)
        k_ref[pl.ds(r0, TR), :] = qkv[D:D + DH].T.astype(BF16)
        vt_ref[:, pl.ds(r0, TR)] = qkv[D + DH:D + 2 * DH].astype(BF16)
        h = _gelu(_dot(_ln(xn).astype(BF16), w1_ref[...]))
        h_ref[pl.ds(pl.multiple_of(r0 + 8, 8), TR), :] = h
        return c
    jax.lax.fori_loop(0, S // TR, p1, 0)

    def p2(t, c):
        r0 = pl.multiple_of(t * TR, TR)
        parts = []
        for j, sh in enumerate((1, -1, 2, -2)):
            win = h_ref[pl.ds(r0, TR + 16), j * 128:(j + 1) * 128]
            parts.append(win[8 - sh:8 - sh + TR].astype(BF16))
        x1 = xn_ref[pl.ds(r0, TR), :] + _dot(jnp.concatenate(parts, axis=1), w2_ref[...])
        l1 = _ln(x1).astype(BF16)
        acc = x1
        for j in range(F // FC):
            a = _gelu(_dot(l1, w3_ref[:, j * FC:(j + 1) * FC]))
            acc = acc + _dot(a.astype(BF16), w4_ref[j * FC:(j + 1) * FC, :])
        g_ref[pl.ds(r0, TR), :] = acc * jax.nn.sigmoid(acc)
        return c
    jax.lax.fori_loop(0, S // TR, p2, 0)

    NU = (S // TQ) * H

    def unit(ref, u):
        return ref.at[pl.ds(pl.multiple_of((u % H) * DH, DH), DH),
                      pl.ds(pl.multiple_of((u // H) * TQ, TQ), TQ)]

    def step(uq, sq, up, sp, m):
        q = unit(qt_ref, uq)[...]
        mx = acc = l = None
        hist = []
        for c in range(S // CK):
            sl = slice(c * CK, (c + 1) * CK)
            s = _dot(k_ref[sl, :], q)
            s_ref[sq, sl, :] = s
            t = _fold8(s, jnp.maximum)
            mx = t if mx is None else jnp.maximum(mx, t)
            hist.append(s[0:8])
            if up is not None:
                mm = jnp.broadcast_to(m, (8, TQ))
                if c >= LAG:
                    mm = jnp.maximum(mm, jnp.minimum(hist[c - LAG], -jnp.inf))
                p = jnp.exp2(s_ref[sp, sl, :] - jnp.tile(mm, (CK // 8, 1)))
                t = _fold8(p, jnp.add)
                l = t if l is None else l + t
                a = _dot(vt_ref[:, sl], p.astype(BF16))
                acc = a if acc is None else acc + a
        if up is not None:
            unit(ot_ref, up)[...] = (acc / jnp.sum(l, axis=0, keepdims=True)).astype(BF16)
        return jnp.max(mx, axis=0, keepdims=True)

    m0 = step(0, 0, None, None, None)

    def p3(i, m):
        for j in range(UNROLL):
            u = UNROLL * i + j
            m = step(jnp.minimum(u + 1, NU - 1), (j + 1) % 2, u, j % 2, m)
        return m
    jax.lax.fori_loop(0, NU // UNROLL, p3, m0)

    def p4(t, c):
        r0 = pl.multiple_of(t * TR, TR)
        o = ot_ref[:, pl.ds(r0, TR)].astype(F32).T.astype(BF16)
        s = _dot(o, wo_ref[...])
        o_ref[pl.ds(r0, TR), :] = (x_ref[pl.ds(r0, TR), :].astype(F32)
                                   + s * g_ref[pl.ds(r0, TR), :]).astype(o_ref.dtype)
        return c
    jax.lax.fori_loop(0, S // TR, p4, 0)


@jax.jit
def pallas_recurrent_scan__grouped_kv_mqa__mixer_s_mlp__prompt_kernel(
    A_x: jax.Array,
    A_wq: jax.Array,
    A_wk: jax.Array,
    A_wv: jax.Array,
    A_wo: jax.Array,
    B_x: jax.Array,
    B_w1: jax.Array,
    B_w2: jax.Array,
    B_w3: jax.Array,
    B_w4: jax.Array,
):
    out = pl.pallas_call(
        _kernel,
        out_shape=jax.ShapeDtypeStruct((S, D), A_x.dtype),
        scratch_shapes=[
            pltpu.VMEM((D + 2 * DH, D), BF16),
            pltpu.VMEM((S, D), F32),
            pltpu.VMEM((S + 16, D), F32),
            pltpu.VMEM((S, D), F32),
            pltpu.VMEM((D, S), BF16),
            pltpu.VMEM((S, DH), BF16),
            pltpu.VMEM((DH, S), BF16),
            pltpu.VMEM((2, S, TQ), F32),
            pltpu.VMEM((D, S), BF16),
        ],
        compiler_params=pltpu.CompilerParams(vmem_limit_bytes=100 * 2**20),
        name="fused_mqa_mixer",
    )(A_x.reshape(S, D), A_wq, A_wk, A_wv, A_wo, B_w1, B_w2, B_w3, B_w4)
    return out.reshape(A_x.shape)
```

```python
import math

import jax
import jax.numpy as jnp
import jax.experimental.pallas as pl
import jax.experimental.pallas.tpu as pltpu

S, D, H, DH, F = 2048, 512, 32, 16, 1792
TQ = 512
CK = 128
TR = 256
FC = 256
UNROLL = 8
LAG = 3
SKEW = 2
G = 128
QSCALE = (DH ** -0.5) * math.log2(math.e)
F32, BF16 = jnp.float32, jnp.bfloat16


def _dot(a, b):
    return jnp.dot(a, b, preferred_element_type=F32)


def _dot_nt(a, b):
    return jax.lax.dot_general(a, b, (((1,), (1,)), ((), ())), preferred_element_type=F32)


def _ln(x):
    m = jnp.mean(x, axis=-1, keepdims=True)
    d = x - m
    v = jnp.mean(d * d, axis=-1, keepdims=True)
    return d * jax.lax.rsqrt(v + 1e-5)


def _gelu(x):
    c = math.sqrt(2.0 / math.pi)
    u = x * (c + (c * 0.044715) * (x * x))
    return (0.5 * x) * (1.0 + jnp.tanh(u))


def _fold8(x, op):
    r = x[0:8]
    for i in range(1, x.shape[0] // 8):
        r = op(r, x[8 * i:8 * i + 8])
    return r


def _aligned(i, n):
    return i * n if isinstance(i, int) else pl.multiple_of(i * n, n)


def _kernel(x_hbm, wq_hbm, wk_hbm, wv_hbm, wo_hbm, w1_hbm, w2_hbm, w3_hbm, w4_hbm, o_hbm,
            x_ref, wq_ref, wk_ref, wv_ref, wo_ref, w1_ref, w2_ref, w3_ref, w4_ref, o_ref,
            wt_ref, xn_ref, xb_ref, lb_ref, h_ref, g_ref, qt_ref, k_ref, vt_ref, s_ref, ot_ref,
            xsem, wsem, osem):
    NT = S // TR

    def xcopy(t):
        rows = pl.ds(_aligned(t, TR), TR)
        return pltpu.make_async_copy(x_hbm.at[rows], x_ref.at[rows], xsem.at[t])

    wcopy = [pltpu.make_async_copy(src, dst, wsem.at[i]) for i, (src, dst) in enumerate((
        (wq_hbm, wq_ref), (wk_hbm, wk_ref), (wv_hbm, wv_ref), (w1_hbm, w1_ref),
        (w2_hbm, w2_ref), (w3_hbm, w3_ref), (w4_hbm, w4_ref), (wo_hbm, wo_ref)))]
    xcopy(0).start()
    for c in wcopy[:4]:
        c.start()
    for t in range(1, NT):
        xcopy(t).start()
    for c in wcopy[4:]:
        c.start()

    h_ref[0:8, :] = jnp.zeros((8, D), F32)
    h_ref[S + 8:S + 16, :] = jnp.zeros((8, D), F32)

    def p1_norm(t):
        rows = pl.ds(_aligned(t, TR), TR)
        xn = _ln(x_ref[rows, :].astype(F32))
        xn_ref[rows, :] = xn
        xb_ref[rows, :] = xn.astype(BF16)
        lb_ref[rows, :] = _ln(xn).astype(BF16)

    def p1_mm(t):
        r0 = _aligned(t, TR)
        rows = pl.ds(r0, TR)
        h = _gelu(_dot(lb_ref[rows, :], w1_ref[...]))
        h_ref[pl.ds(r0 + 8 if isinstance(r0, int) else pl.multiple_of(r0 + 8, 8), TR), :] = h
        qkv = _dot_nt(wt_ref[...], xb_ref[rows, :])
        k_ref[rows, :] = qkv[0:DH].T.astype(BF16)
        vt_ref[:, rows] = qkv[DH:2 * DH].astype(BF16)
        qt_ref[:, rows] = (qkv[2 * DH:] * QSCALE).astype(BF16)

    xcopy(0).wait()
    p1_norm(0)
    for c in wcopy[:3]:
        c.wait()
    wt_ref[0:DH, :] = wk_ref[...]
    wt_ref[DH:2 * DH, :] = wv_ref[...]
    wt_ref[2 * DH:, :] = wq_ref[...].astype(F32).T.astype(BF16)
    wcopy[3].wait()

    def p1(t, c):
        xcopy(t + 1).wait()
        p1_mm(t)
        p1_norm(t + 1)
        return c
    with jax.named_scope('p1'):
        jax.lax.fori_loop(0, NT - 1, p1, 0)

    def p2_mix(t):
        r0 = _aligned(t, TR)
        rows = pl.ds(r0, TR)
        parts = []
        for j, sh in enumerate((1, -1, 2, -2)):
            win = h_ref[pl.ds(r0, TR + 16), j * 128:(j + 1) * 128]
            parts.append(win[8 - sh:8 - sh + TR].astype(BF16))
        x1 = xn_ref[rows, :] + _dot(jnp.concatenate(parts, axis=1), w2_ref[...])
        g_ref[rows, :] = x1
        lb_ref[rows, :] = _ln(x1).astype(BF16)

    def p2_mlp(t, mid=None):
        rows = pl.ds(_aligned(t, TR), TR)
        l1 = lb_ref[rows, :]
        acc = g_ref[rows, :]
        nf = F // FC
        a = _dot(l1, w3_ref[:, 0:FC])
        if mid is not None:
            mid()
        for j in range(nf):
            nxt = _dot(l1, w3_ref[:, (j + 1) * FC:(j + 2) * FC]) if j + 1 < nf else None
            acc = acc + _dot(_gelu(a).astype(BF16), w4_ref[j * FC:(j + 1) * FC, :])
            a = nxt
        g_ref[rows, :] = acc

    wcopy[4].wait()
    p2_mix(0)
    p1_mm(NT - 1)
    wcopy[5].wait()
    wcopy[6].wait()

    def p2(t, c):
        p2_mlp(t, lambda: p2_mix(jnp.minimum(t + 1, NT - 1)))
        return c
    with jax.named_scope('p2'):
        jax.lax.fori_loop(0, NT, p2, 0)

    NU = (S // TQ) * H

    NC = S // CK

    def q_of(u):
        return qt_ref[pl.ds(_aligned(u % H, DH), DH), pl.ds(_aligned(u // H, TQ), TQ)]

    def qk(q, slot, c, mx):
        sl = slice(c * CK, (c + 1) * CK)
        s = _dot(k_ref[sl, :], q)
        s_ref[slot, sl, :] = s
        t = _fold8(s, jnp.maximum)
        return (t if mx is None else jnp.maximum(mx, t)), [s[g:g + 8, 0:128] for g in range(0, CK, G)]

    def colmax(mx):
        return jnp.broadcast_to(jnp.max(mx, axis=0, keepdims=True), (8, TQ))

    def pv(slot, c, m, acc, l, dep):
        sl = slice(c * CK, (c + 1) * CK)
        if dep is not None:
            mm = jnp.concatenate(
                [jnp.tile(jnp.maximum(m, jnp.tile(jnp.minimum(d, -jnp.inf), (1, TQ // 128))), (G // 8, 1))
                 for d in dep], axis=0)
        else:
            mm = jnp.tile(m, (CK // 8, 1))
        p = jnp.exp2(s_ref[slot, sl, :] - mm)
        t = _fold8(p, jnp.add)
        a = _dot(vt_ref[:, sl], p.astype(BF16))
        return (a, t) if c == 0 else (acc + a, l + t)

    def put(u, acc, l):
        row = jnp.where(u < 0, H, u % H)
        col = jnp.maximum(u, 0) // H
        ot_ref[pl.ds(_aligned(row, DH), DH), pl.ds(_aligned(col, TQ), TQ)] = (
            acc / jnp.sum(l, axis=0, keepdims=True)).astype(BF16)

    s_ref[1, (NC - SKEW) * CK:, :] = jnp.zeros((SKEW * CK, TQ), F32)
    mx = None
    for c in range(NC):
        mx, _ = qk(q_of(0), 0, c, mx)
    zero = jnp.zeros((8, TQ), F32)
    carry0 = (zero, colmax(mx), jnp.zeros((DH, TQ), F32), zero)

    def p3(i, carry):
        m_old, m_cur, acc, l = carry
        hist = []
        for j in range(UNROLL):
            u = UNROLL * i + j
            q = q_of(jnp.minimum(u + 1, NU - 1))
            mx = None
            for c in range(NC):
                mx, tag = qk(q, (j + 1) % 2, c, mx)
                hist.append(tag)
                dep = hist[-1 - LAG] if len(hist) > LAG else None
                if c < SKEW:
                    acc, l = pv((j + 1) % 2, NC - SKEW + c, m_old, acc, l, dep)
                    if c == SKEW - 1:
                        put(u - 1, acc, l)
                else:
                    acc, l = pv(j % 2, c - SKEW, m_cur, acc, l, dep)
            m_old, m_cur = m_cur, colmax(mx)
        return m_old, m_cur, acc, l

    def ocopy(t):
        rows = pl.ds(_aligned(t, TQ), TQ)
        return pltpu.make_async_copy(o_ref.at[rows], o_hbm.at[rows], osem.at[t])

    def p4(t):
        rows = pl.ds(_aligned(t, TQ), TQ)
        o = ot_ref[0:D, rows].astype(F32).T.astype(BF16)
        b = g_ref[rows, :]
        s = _dot(o, wo_ref[...])
        o_ref[rows, :] = (x_ref[rows, :].astype(F32) + s * (b * jax.nn.sigmoid(b))).astype(o_ref.dtype)
        ocopy(t).start()

    wcopy[7].wait()
    n_in = H // UNROLL

    def tile(t, m):
        with jax.named_scope('p3'):
            m = jax.lax.fori_loop(t * n_in, (t + 1) * n_in, p3, m)
        with jax.named_scope('p4'):
            pl.when(t > 0)(lambda: p4(jnp.maximum(t - 1, 0)))
        return m
    m_old, _, acc, l = jax.lax.fori_loop(0, S // TQ, tile, carry0)
    for c in range(NC - SKEW, NC):
        acc, l = pv((NU - 1) % 2, c, m_old, acc, l, None)
    put(NU - 1, acc, l)
    p4(S // TQ - 1)
    for t in range(S // TQ):
        ocopy(t).wait()


@jax.jit
def pallas_recurrent_scan__grouped_kv_mqa__mixer_s_mlp__prompt_kernel(
    A_x: jax.Array,
    A_wq: jax.Array,
    A_wk: jax.Array,
    A_wv: jax.Array,
    A_wo: jax.Array,
    B_x: jax.Array,
    B_w1: jax.Array,
    B_w2: jax.Array,
    B_w3: jax.Array,
    B_w4: jax.Array,
):
    out = pl.pallas_call(
        _kernel,
        out_shape=jax.ShapeDtypeStruct((S, D), A_x.dtype),
        in_specs=[pl.BlockSpec(memory_space=pl.ANY)] * 9,
        out_specs=pl.BlockSpec(memory_space=pl.ANY),
        scratch_shapes=[
            pltpu.VMEM((S, D), BF16), pltpu.VMEM((D, D), BF16),
            pltpu.VMEM((DH, D), BF16), pltpu.VMEM((DH, D), BF16),
            pltpu.VMEM((D, D), BF16), pltpu.VMEM((D, D), BF16), pltpu.VMEM((D, D), BF16),
            pltpu.VMEM((D, F), BF16), pltpu.VMEM((F, D), BF16), pltpu.VMEM((S, D), BF16),
            pltpu.VMEM((D + 2 * DH, D), BF16),
            pltpu.VMEM((S, D), F32),
            pltpu.VMEM((S, D), BF16),
            pltpu.VMEM((S, D), BF16),
            pltpu.VMEM((S + 16, D), F32),
            pltpu.VMEM((S, D), F32),
            pltpu.VMEM((D, S), BF16),
            pltpu.VMEM((S, DH), BF16),
            pltpu.VMEM((DH, S), BF16),
            pltpu.VMEM((2, S, TQ), F32),
            pltpu.VMEM((D + DH, S), BF16),
            pltpu.SemaphoreType.DMA((S // TR,)),
            pltpu.SemaphoreType.DMA((8,)),
            pltpu.SemaphoreType.DMA((S // TQ,)),
        ],
        compiler_params=pltpu.CompilerParams(vmem_limit_bytes=100 * 2**20),
        name="fused_mqa_mixer",
    )(A_x.reshape(S, D), A_wq, A_wk.T, A_wv.T, A_wo, B_w1, B_w2, B_w3, B_w4)
    return out.reshape(A_x.shape)
```
